```python
import jax
import jax.numpy as jnp

def _softmax(x, axis=-1):
    return jax.nn.softmax(x, axis=axis)

def _gelu(x):
    return jax.nn.gelu(x, approximate=True)

def _silu(x):
    return jax.nn.silu(x)

def _sigmoid(x):
    return jax.nn.sigmoid(x)

def _layernorm(x, axis=-1, eps=1e-05):
    m = jnp.mean(x, axis=axis, keepdims=True)
    v = jnp.var(x, axis=axis, keepdims=True)
    return (x - m) / jnp.sqrt(v + eps)

def _scatter_add(tgt, idx, src, axis=0):
    return tgt.at[idx].add(src)

def _segment_sum(src, seg, n):
    return jax.ops.segment_sum(src, seg, n)

class _Rng:

    def __init__(self, key):
        self._k = key

    def _next(self):
        self._k, sub = jax.random.split(self._k)
        return sub

    def normal(self, shape):
        return jax.random.normal(self._next(), shape, dtype=jnp.bfloat16)

    def randint(self, lo, hi, shape):
        return jax.random.randint(self._next(), shape, lo, hi, dtype=jnp.int32)

    def uniform(self, shape, lo=0.0, hi=1.0):
        return jax.random.uniform(self._next(), shape, jnp.bfloat16, lo, hi)

    def permutation(self, n):
        return jax.random.permutation(self._next(), n)
kernel_name = 'standalone__window_attn_davit__vision'

def setup_inputs():
    _rng = _Rng(jax.random.key(int.from_bytes(__import__("os").urandom(4), "little")))
    _w = lambda a: (lambda t: t.astype(jnp.bfloat16) if jnp.issubdtype(t.dtype, jnp.floating) else t)(jnp.asarray(a))
    HW = 512
    C0 = 192
    ws = 7
    nh = 4
    H = W = max(HW // ws * ws, ws)
    C = max(C0 // nh * nh, nh)
    k = 3
    return {'x': _w((lambda *s: _rng.normal(s) * 0.05)(1, H, W, C)), 'dw_pe': _w((lambda *s: _rng.normal(s) * 0.05)(k, k, C) * 0.1), 'w_qkv': _w((lambda *s: _rng.normal(s) * 0.05)(C, 3 * C) * C ** (-0.5)), 'w_o': _w((lambda *s: _rng.normal(s) * 0.05)(C, C) * C ** (-0.5))}

def reference(x, dw_pe, w_qkv, w_o):
    B, H, W, C = x.shape
    ws = 7
    nh = 4
    dh = C // nh
    kk = dw_pe.shape[0]
    pad = kk // 2
    xp = jnp.pad(x, ((0, 0), (pad, pad), (pad, pad), (0, 0)))
    pe = jnp.zeros_like(x)
    for i in range(kk):
        for j in range(kk):
            pe = pe + xp[:, i:i + H, j:j + W, :] * dw_pe[i, j][None, None, None, :]
    x0 = x + pe
    h = _layernorm(x0, axis=-1)
    hw = h.reshape(B, H // ws, ws, W // ws, ws, C)
    hw = (lambda x, *d: x.transpose(*d))(hw, 0, 1, 3, 2, 4, 5)
    hw = hw.reshape(-1, ws * ws, C)
    qkv = (hw @ w_qkv).reshape(-1, ws * ws, 3, nh, dh)
    q = qkv[:, :, 0].copy()
    k = qkv[:, :, 1].copy()
    v = qkv[:, :, 2].copy()
    scale = dh ** (-0.5)
    attn = jnp.einsum('wnhd,wmhd->whnm', q, k) * scale
    attn = _softmax(attn, axis=-1)
    out = jnp.einsum('whnm,wmhd->wnhd', attn, v)
    out = out.reshape(-1, ws * ws, C) @ w_o
    out = out.reshape(B, H // ws, W // ws, ws, ws, C)
    out = (lambda x, *d: x.transpose(*d))(out, 0, 1, 3, 2, 4, 5)
    out = out.reshape(B, H, W, C)
    return x0 + out
```

```python
import functools
import numpy as np
import jax
import jax.numpy as jnp
from jax.experimental import pallas as pl
from jax.experimental.pallas import tpu as pltpu

WS = 7
NH = 4
C = 192
DH = 48
F32 = jnp.float32
BF16 = jnp.bfloat16
NN = (((1,), (0,)), ((), ()))
NT = (((1,), (1,)), ((), ()))
LOG2E = 1.4426950408889634


def _dot(a, b, d):
    return jax.lax.dot_general(a, b, d, preferred_element_type=F32)


def _iota(shape, dim):
    return jax.lax.broadcasted_iota(jnp.int32, shape, dim)


def _kernel(x_ref, xu_ref, xd_ref, dw_ref, wqkv_ref, wo_ref, o_ref,
            wb_ref, wk_ref, wqv_ref, wot_ref, x0_ref, hna_ref, hnb_ref, osa_ref, osb_ref,
            kna_ref, knb_ref, qva_ref, qvb_ref, ota_ref, otb_ref, *, W, W2, nstrip):
    s = pl.program_id(0)

    @pl.when(s == 0)
    def _prep():
        dw = dw_ref[...].astype(F32)
        dwp = jnp.concatenate([dw, jnp.zeros((128 - 9, C), F32)], axis=0)
        dwt = dwp.T
        for t in range(9):
            col = dwt[:, t:t + 1]
            if t == 4:
                col = col + 1.0
            wb_ref[t] = jnp.broadcast_to(col, (C, 128))
        w = wqkv_ref[...].astype(F32)
        z = jnp.zeros((C, 32), F32)
        wk = jnp.concatenate([w[:, C:C + 96], z, w[:, C + 96:2 * C], z], axis=1)
        wkp = jnp.concatenate([wk, jnp.zeros((64, 256), F32)], axis=0)
        wk_ref[0] = wkp[0:128].astype(BF16)
        wk_ref[1] = wkp[128:256].astype(BF16)
        wq = w[:, 0:C] * (DH ** -0.5 * LOG2E)
        wqv = jnp.concatenate([wq, w[:, 2 * C:3 * C]], axis=1)
        wqv = jnp.concatenate([wqv, jnp.zeros((64, 2 * C), F32)], axis=0)
        wqv_ref[0] = wqv[0:128].T.astype(BF16)
        wqv_ref[1] = wqv[128:256].T.astype(BF16)
        wo = wo_ref[...].astype(F32)
        wo = jnp.concatenate([wo, jnp.zeros((C, 64), F32)], axis=1)
        wot_ref[0] = wo[0:128].T[0:C].astype(BF16)
        wo1 = jnp.concatenate([jnp.zeros((64, 256), F32), wo[128:C]], axis=0)
        wot_ref[1] = wo1.T[0:C].astype(BF16)
        for r_ in (kna_ref, knb_ref, qva_ref, qvb_ref, ota_ref, otb_ref):
            r_[...] = jnp.zeros(r_.shape, F32)
        for r_ in (hna_ref, hnb_ref, osa_ref, osb_ref, x0_ref):
            r_[...] = jnp.zeros(r_.shape, F32)

    lane = _iota((1, W2), 1)
    cmask = lane < W

    def load_row(r, c0, nc):
        if r == 0:
            v = xu_ref[0, 0, pl.ds(c0, nc), :]
            v = jnp.where(jnp.logical_and(cmask, s > 0), v, jnp.zeros_like(v))
        elif r == 8:
            v = xd_ref[0, 0, pl.ds(c0, nc), :]
            v = jnp.where(jnp.logical_and(cmask, s < nstrip - 1), v, jnp.zeros_like(v))
        else:
            v0 = x_ref[0, r - 1, pl.ds(c0, nc), 0:W2 - 128]
            v1 = x_ref[0, r - 1, pl.ds(c0, nc), W2 - 128:W2]
            v1 = jnp.where(cmask[:, W2 - 128:], v1, jnp.zeros_like(v1))
            v = jnp.concatenate([v0, v1], axis=1)
        return v

    CG = 16

    def conv_item(g, xs):
        c0 = pl.multiple_of(g * CG, CG)
        wts = [wb_ref[t, pl.ds(c0, CG), :] for t in range(9)]
        wts = [jnp.concatenate([w_] * (W2 // 128), axis=1) for w_ in wts]
        acc = [None] * WS
        for r in range(9):
            v = load_row(r, c0, CG)
            sh = [pltpu.roll(v, 1, 1).astype(F32), v.astype(F32), pltpu.roll(v, W2 - 1, 1).astype(F32)]
            for a in range(3):
                i = r - a
                if i < 0 or i >= WS:
                    continue
                t = sh[0] * wts[3 * a] + sh[1] * wts[3 * a + 1] + sh[2] * wts[3 * a + 2]
                acc[i] = t if acc[i] is None else acc[i] + t
                if a == 2:
                    x0_ref[xs, i, pl.ds(c0, CG), :] = acc[i]


    def ln_item(i, xs, hn_ref):
        for t in range(W2 // 128):
            x0 = x0_ref[xs, i, :, t * 128:(t + 1) * 128]
            m = jnp.sum(x0, axis=0, keepdims=True) * (1.0 / C)
            xc = x0 - m
            var = jnp.sum(xc * xc, axis=0, keepdims=True) * (1.0 / C)
            h = xc * jax.lax.rsqrt(var + 1e-5)
            ht = h.T
            hn_ref[i, 0, t * 128:(t + 1) * 128, :] = ht[:, 0:128]
            hn_ref[i, 1, t * 128:(t + 1) * 128, 0:64] = ht[:, 128:C]

    R = 8 * WS
    lane128 = _iota((R, 128), 1)
    l_lt48 = lane128 < DH
    lane112 = _iota((R, 2 * R), 1)
    l_lt56 = lane112 < R
    rowvalid = (_iota((R, 2 * R), 0) & 7) != 7
    mq = (_iota((2 * DH, 2 * R), 0) < DH) == (_iota((2 * DH, 2 * R), 1) < R)
    l_lt56_d = _iota((DH, 2 * R), 1) < R
    NP = (W // WS + 1) // 2

    def stage_a(u, kn_ref, qv_ref, hn_ref):
        ca = u * (2 * WS)
        cb = ca + WS
        hw0 = jnp.concatenate([hn_ref[i, 0, pl.ds(c_, 8), :] for c_ in (ca, cb) for i in range(WS)], axis=0)
        hw1 = jnp.concatenate([hn_ref[i, 1, pl.ds(c_, 8), :] for c_ in (ca, cb) for i in range(WS)], axis=0)
        kn_ref[...] = _dot(hw0, wk_ref[0], NN) + _dot(hw1, wk_ref[1], NN)
        qv_ref[...] = _dot(wqv_ref[0], hw0, NT) + _dot(wqv_ref[1], hw1, NT)

    def stage_s(kn_ref, qv_ref):
        sts = []
        for p in range(2):
            qp = qv_ref[96 * p:96 * p + 96, :]
            ka = kn_ref[0:R, 128 * p:128 * p + 128]
            kb = kn_ref[R:2 * R, 128 * p:128 * p + 128]
            lx = jnp.where(l_lt48, ka, kb)[:, 0:96]
            ly = jnp.where(l_lt48, kb, ka)[:, 0:96]
            rx = jnp.where(mq, qp, 0.0)
            ry = jnp.where(mq, 0.0, qp)
            sts.append(_dot(lx, rx, NN))
            sts.append(_dot(ly, ry, NN))
        return sts

    def stage_pv(sts, qv_ref, ot_ref):
        outs = []
        for p in range(2):
            vp = qv_ref[C + 96 * p:C + 96 * p + 96, :]
            res = []
            for (st, v_lo, v_hi) in ((sts[2 * p], vp[0:DH], vp[DH:2 * DH]), (sts[2 * p + 1], vp[DH:2 * DH], vp[0:DH])):
                st = jnp.where(rowvalid, st, -jnp.inf)
                mx = jnp.max(st, axis=0, keepdims=True)
                pt = jnp.exp2(st - mx)
                l = jnp.sum(pt, axis=0, keepdims=True)
                rhs = jnp.concatenate([jnp.where(l_lt56, pt, 0.0), jnp.where(l_lt56, 0.0, pt)], axis=0)
                lv = jnp.where(l_lt56_d, v_lo, v_hi)
                o = _dot(lv, rhs, NN)
                res.append(o * (1.0 / l))
            outs.append(jnp.where(l_lt56_d, res[0], res[1]))
            outs.append(jnp.where(l_lt56_d, res[1], res[0]))
        ot_ref[:, 0:2 * R] = jnp.concatenate(outs, axis=0)

    def stage_d(u, ot_ref, os_ref):
        ca = u * (2 * WS)
        cb = ca + WS
        on0 = ot_ref[0:128, :].T
        on1 = ot_ref[64:192, :].T
        for c_, r0 in ((ca, 0), (cb, R)):
            for i in range(WS):
                os_ref[i, 0, pl.ds(c_, WS), :] = on0[r0 + 8 * i:r0 + 8 * i + WS, :]
                os_ref[i, 1, pl.ds(c_, WS), :] = on1[r0 + 8 * i:r0 + 8 * i + WS, :]

    def half(u, rd, wr, hn_ref, os_ref):
        kn_r, qv_r, ot_r = rd
        kn_w, qv_w, ot_w = wr
        stage_d(jnp.where(u >= 1, u - 1, NP + 1), ot_w, os_ref)
        sts = stage_s(kn_r, qv_r)
        stage_a(jnp.minimum(u + 1, NP), kn_w, qv_w, hn_ref)
        stage_pv(sts, qv_r, ot_r)

    bufa = (kna_ref, qva_ref, ota_ref)
    bufb = (knb_ref, qvb_ref, otb_ref)
    def out_item(i, xs, os_ref):
        for t in range(W2 // 128):
            y = (_dot(wot_ref[0], os_ref[i, 0, t * 128:(t + 1) * 128, :], NT)
                 + _dot(wot_ref[1], os_ref[i, 1, t * 128:(t + 1) * 128, :], NT))
            y = y + x0_ref[xs, i, :, t * 128:(t + 1) * 128]
            o_ref[0, i, :, t * 128:(t + 1) * 128] = y.astype(o_ref.dtype)

    NCONV = C // CG
    assert NP % 2 == 1 and NP // 2 + 1 == NCONV + WS
    xs_w = jax.lax.rem(s, 3)
    xs_o = jax.lax.rem(s + 1, 3)

    def body(hn_r, hn_w, os_w, os_r):
        stage_a(0, kna_ref, qva_ref, hn_r)

        def loop1(it, carry):
            conv_item(it, xs_w)
            half(2 * it, bufa, bufb, hn_r, os_w)
            half(2 * it + 1, bufb, bufa, hn_r, os_w)
            return carry

        jax.lax.fori_loop(0, NCONV, loop1, 0)

        def loop2(it, carry):
            out_item(it, xs_o, os_r)
            ln_item(it, xs_w, hn_w)
            half(2 * (it + NCONV), bufa, bufb, hn_r, os_w)
            half(2 * (it + NCONV) + 1, bufb, bufa, hn_r, os_w)
            return carry

        jax.lax.fori_loop(0, WS, loop2, 0)

    par = jax.lax.rem(s, 2)

    @pl.when(par == 0)
    def _():
        body(hna_ref, hnb_ref, osa_ref, osb_ref)

    @pl.when(par == 1)
    def _():
        body(hnb_ref, hna_ref, osb_ref, osa_ref)


@jax.jit
def pallas_standalone__window_attn_davit__vision_kernel(x: jax.Array, dw_pe: jax.Array, w_qkv: jax.Array, w_o: jax.Array):
    B, H, W, Cc = x.shape
    assert B == 1 and Cc == C and H % WS == 0 and W % WS == 0
    W2 = -(-W // 128) * 128
    nstrip = H // WS
    xt = x.transpose(0, 1, 3, 2)
    dw = dw_pe.reshape(9, C)
    RP = W2 + 40
    out = pl.pallas_call(
        functools.partial(_kernel, W=W, W2=W2, nstrip=nstrip),
        grid=(nstrip + 2,),
        in_specs=[
            pl.BlockSpec((1, WS, C, W2), lambda s: (0, jnp.minimum(s, nstrip - 1), 0, 0)),
            pl.BlockSpec((1, 1, C, W2), lambda s: (0, jnp.clip(s * WS - 1, 0, H - 1), 0, 0)),
            pl.BlockSpec((1, 1, C, W2), lambda s: (0, jnp.minimum(s * WS + WS, H - 1), 0, 0)),
            pl.BlockSpec((9, C), lambda s: (0, 0)),
            pl.BlockSpec((C, 3 * C), lambda s: (0, 0)),
            pl.BlockSpec((C, C), lambda s: (0, 0)),
        ],
        out_specs=pl.BlockSpec((1, WS, C, W2), lambda s: (0, jnp.maximum(s - 2, 0), 0, 0)),
        out_shape=jax.ShapeDtypeStruct((1, H, C, W), x.dtype),
        scratch_shapes=[
            pltpu.VMEM((9, C, 128), F32),
            pltpu.VMEM((2, 128, 256), BF16),
            pltpu.VMEM((2, 2 * C, 128), BF16),
            pltpu.VMEM((2, C, 128), BF16),
            pltpu.VMEM((3, WS, C, W2), F32),
            pltpu.VMEM((WS, 2, RP, 128), F32),
            pltpu.VMEM((WS, 2, RP, 128), F32),
            pltpu.VMEM((WS, 2, RP, 128), F32),
            pltpu.VMEM((WS, 2, RP, 128), F32),
            pltpu.VMEM((112, 256), F32), pltpu.VMEM((112, 256), F32),
            pltpu.VMEM((2 * C, 112), F32), pltpu.VMEM((2 * C, 112), F32),
            pltpu.VMEM((C, 128), F32), pltpu.VMEM((C, 128), F32),
        ],
        compiler_params=pltpu.CompilerParams(
            dimension_semantics=("arbitrary",), vmem_limit_bytes=100 * 2**20),
        name="davit_window_attn",
    )(xt, xt, xt, dw, w_qkv, w_o)
    return out.transpose(0, 1, 3, 2)
```

```python
import functools
import jax
import jax.numpy as jnp
from jax.experimental import pallas as pl
from jax.experimental.pallas import tpu as pltpu

WS = 7
NH = 4
C = 192
DH = 48
F32 = jnp.float32
BF16 = jnp.bfloat16
NN = (((1,), (0,)), ((), ()))
NT = (((1,), (1,)), ((), ()))
LOG2E = 1.4426950408889634
HORD = 'vsda'
NB1 = 2
CY = 3
U32 = jnp.uint32


def _pk(w):
    return pltpu.bitcast(w.astype(BF16), U32)


def _unpk(w):
    return pltpu.bitcast(w, BF16)


def _dot(a, b, d):
    return jax.lax.dot_general(a, b, d, preferred_element_type=F32)


def _iota(shape, dim):
    return jax.lax.broadcasted_iota(jnp.int32, shape, dim)


def _interleave(*streams):
    items = [[g, n, 0] for g, n in streams]
    while items:
        it = min(items, key=lambda t: (t[2] + 0.5) / t[1])
        try:
            next(it[0])
            it[2] += 1
        except StopIteration:
            items.remove(it)


def _chain(*gens):
    for g in gens:
        yield from g


def _kernel(x_ref, xu_ref, xd_ref, dw_ref, wqkv_ref, wo_ref, o_ref,
            wb_ref, wk_ref, wqv_ref, wot_ref, x0_ref, hna_ref, hnb_ref, osa_ref, osb_ref,
            xsa_ref, xsb_ref, kna_ref, knb_ref, q0, q1, v0, v1, p0, p1, rl0, rl1, ot0, ot1, *, W, W2, nstrip):
    s = pl.program_id(0)
    q_ref, v_ref, p_ref, rl_ref, ot_ref = (q0, q1), (v0, v1), (p0, p1), (rl0, rl1), (ot0, ot1)

    @pl.when(s == 0)
    def _prep():
        dw = dw_ref[...].astype(F32)
        dwp = jnp.concatenate([dw, jnp.zeros((128 - 9, C), F32)], axis=0)
        dwt = dwp.T
        for t in range(9):
            col = dwt[:, t:t + 1]
            if t == 4:
                col = col + 1.0
            wb_ref[t] = jnp.broadcast_to(col, (C, 128))
        w = wqkv_ref[...].astype(F32)
        z = jnp.zeros((C, 32), F32)
        wk = jnp.concatenate([w[:, C:C + 96], z, w[:, C + 96:2 * C], z], axis=1)
        wkp = jnp.concatenate([wk[0:128], jnp.zeros((64, 256), F32), wk[128:C]], axis=0)
        for kt in range(2):
            for nt in range(2):
                wk_ref[kt, nt] = _pk(wkp[128 * kt:128 * kt + 128, 128 * nt:128 * nt + 128])
        wq = w[:, 0:C] * (DH ** -0.5 * LOG2E)
        wqv = jnp.concatenate([wq, w[:, 2 * C:3 * C]], axis=1)
        wqv = jnp.concatenate([wqv[0:128], jnp.zeros((64, 2 * C), F32), wqv[128:C]], axis=0)
        wqv_ref[0] = _pk(wqv[0:128].T)
        wqv_ref[1] = _pk(wqv[128:256].T)
        wo = wo_ref[...].astype(F32)
        wo = jnp.concatenate([wo, jnp.zeros((C, 64), F32)], axis=1)
        wot_ref[0] = _pk(wo[0:128].T[0:C])
        wo1 = jnp.concatenate([jnp.zeros((64, 256), F32), wo[128:C]], axis=0)
        wot_ref[1] = _pk(wo1.T[0:C])
        for r_ in (kna_ref, knb_ref, q0, q1, v0, v1, p0, p1, rl0, rl1, ot0, ot1):
            r_[...] = jnp.zeros(r_.shape, F32)
        for r_ in (hna_ref, hnb_ref, osa_ref, osb_ref, x0_ref):
            r_[...] = jnp.zeros(r_.shape, F32)
        for r_ in (xsa_ref, xsb_ref):
            r_[...] = jnp.zeros(r_.shape, BF16)

    lane = _iota((1, W2), 1)
    cmask = lane < W

    def load_row(r, c0, nc):
        if r == 0:
            v = xu_ref[0, 0, pl.ds(c0, nc), :]
            v = jnp.where(jnp.logical_and(cmask, s > 0), v, jnp.zeros_like(v))
        elif r == 8:
            v = xd_ref[0, 0, pl.ds(c0, nc), :]
            v = jnp.where(jnp.logical_and(cmask, s < nstrip - 1), v, jnp.zeros_like(v))
        else:
            v0 = x_ref[0, r - 1, pl.ds(c0, nc), 0:W2 - 128]
            v1 = x_ref[0, r - 1, pl.ds(c0, nc), W2 - 128:W2]
            v1 = jnp.where(cmask[:, W2 - 128:], v1, jnp.zeros_like(v1))
            v = jnp.concatenate([v0, v1], axis=1)
        return v

    CG = 16

    RG = 32

    def roll_gen(it, xs_ref):
        c0 = it * RG
        for r in range(9):
            v = load_row(r, c0, RG)
            xs_ref[1, r, pl.ds(c0, RG), :] = v
            xs_ref[0, r, pl.ds(c0, RG), :] = pltpu.roll(v, 1, 1)
            yield
            xs_ref[2, r, pl.ds(c0, RG), :] = pltpu.roll(v, W2 - 1, 1)
            yield
    N_ROLL = 18

    def conv_gen(g, xs, xs_ref):
        for t in range(W2 // 128):
            ts = slice(t * 128, (t + 1) * 128)
            for hh in range(CG // 8):
                c0 = g * CG + 8 * hh
                if not isinstance(c0, int):
                    c0 = pl.multiple_of(c0, 8)
                wts = [wb_ref[k_, pl.ds(c0, 8), :] for k_ in range(9)]
                acc = [None] * WS
                for r in range(9):
                    sh = [xs_ref[j, r, pl.ds(c0, 8), ts].astype(F32) for j in range(3)]
                    for a in range(3):
                        i = r - a
                        if i < 0 or i >= WS:
                            continue
                        t_ = sh[0] * wts[3 * a] + sh[1] * wts[3 * a + 1] + sh[2] * wts[3 * a + 2]
                        acc[i] = t_ if acc[i] is None else acc[i] + t_
                        if a == 2:
                            x0_ref[xs, i, pl.ds(c0, 8), ts] = acc[i]
                    if r % CY == CY - 1:
                        yield
    N_CONV = 4 * (CG // 8) * (9 // CY)

    def ln_gen(i, xs, hn_ref):
        for t in range(W2 // 128):
            x0 = x0_ref[xs, i, :, t * 128:(t + 1) * 128]
            m = jnp.sum(x0, axis=0, keepdims=True) * (1.0 / C)
            yield
            xc = x0 - m
            var = jnp.sum(xc * xc, axis=0, keepdims=True) * (1.0 / C)
            yield
            h = xc * jax.lax.rsqrt(var + 1e-5)
            ht0 = h[0:128].T
            yield
            hn_ref[i, 0, t * 128:(t + 1) * 128, :] = ht0
            ht1 = h[64:C].T
            yield
            hn_ref[i, 1, t * 128:(t + 1) * 128, :] = ht1
            yield
    N_LN = 5 * 4

    def kproj_gen(i, hn_ref, kn_ref):
        for t in range(W2 // 128):
            ht0 = hn_ref[i, 0, t * 128:(t + 1) * 128, :]
            ht1 = hn_ref[i, 1, t * 128:(t + 1) * 128, :]
            d = []
            for nt in range(2):
                d.append(_dot(ht0, _unpk(wk_ref[0, nt]), NN))
                yield
                d.append(_dot(ht1, _unpk(wk_ref[1, nt]), NN))
                yield
            for nt in range(2):
                kn_ref[i, nt, t * 128:(t + 1) * 128, :] = d[2 * nt] + d[2 * nt + 1]
                yield
    N_KP = 6 * 4

    def out_gen(i, xs, os_ref):
        for t in range(W2 // 128):
            y0 = _dot(_unpk(wot_ref[0]), os_ref[i, 0, t * 128:(t + 1) * 128, :], NT)
            yield
            y1 = _dot(_unpk(wot_ref[1]), os_ref[i, 1, t * 128:(t + 1) * 128, :], NT)
            yield
            y = (y0 + y1) + x0_ref[xs, i, :, t * 128:(t + 1) * 128]
            o_ref[0, i, :, t * 128:(t + 1) * 128] = y.astype(o_ref.dtype)
            yield
    N_OUT = 3 * 4

    R = 8 * WS
    lane128 = _iota((R, 128), 1)
    l_lt48 = lane128 < DH
    lane112 = _iota((R, 2 * R), 1)
    l_lt56 = lane112 < R
    rowvalid = (_iota((R, 2 * R), 0) & 7) != 7
    mq = (_iota((2 * DH, 2 * R), 0) < DH) == (_iota((2 * DH, 2 * R), 1) < R)
    l_lt56_d = _iota((DH, 2 * R), 1) < R
    NP = (W // WS + 1) // 2

    def gen_a(u, part, dst_ref, hn_ref):
        ca = u * (2 * WS)
        cb = ca + WS
        hw0 = jnp.concatenate([hn_ref[i, 0, pl.ds(c_, 8), :] for c_ in (ca, cb) for i in range(WS)], axis=0)
        hw1 = jnp.concatenate([hn_ref[i, 1, pl.ds(c_, 8), :] for c_ in (ca, cb) for i in range(WS)], axis=0)
        hf = C // 2
        d0 = _dot(_unpk(wqv_ref[0, part * hf:(part + 1) * hf]), hw0, NT)
        yield
        d1 = _dot(_unpk(wqv_ref[1, part * hf:(part + 1) * hf]), hw1, NT)
        yield
        return d0, d1, dst_ref

    def gen_aa(uq, slq, uv, slv, hn_ref):
        rq = rv = None
        if uq is not None:
            rq = yield from gen_a(uq, 0, q_ref[slq], hn_ref)
        if uv is not None:
            rv = yield from gen_a(uv, 1, v_ref[slv], hn_ref)
        if rq is not None:
            rq[2][...] = rq[0] + rq[1]
        yield
        if rv is not None:
            rv[2][...] = rv[0] + rv[1]
        yield

    def gen_s(u, sl, kn_ref):
        if not isinstance(u, int):
            u = jnp.maximum(u, 0)
        ca = u * (2 * WS)
        cb = ca + WS
        sts = []
        for p in range(2):
            qp = q_ref[sl][96 * p:96 * p + 96, :]
            ka = jnp.concatenate([kn_ref[i, p, pl.ds(ca, 8), :] for i in range(WS)], axis=0)
            kb = jnp.concatenate([kn_ref[i, p, pl.ds(cb, 8), :] for i in range(WS)], axis=0)
            lx = jnp.where(l_lt48, ka, kb)[:, 0:96]
            rx = jnp.where(mq, qp, 0.0)
            sts.append(_dot(lx, rx, NN))
            yield
            ly = jnp.where(l_lt48, kb, ka)[:, 0:96]
            ry = jnp.where(mq, 0.0, qp)
            sts.append(_dot(ly, ry, NN))
            yield
        for n, st in enumerate(sts):
            st = jnp.where(rowvalid, st, -jnp.inf)
            mx = jnp.max(st, axis=0, keepdims=True)
            pt = jnp.exp2(st - mx)
            l = jnp.sum(pt, axis=0, keepdims=True)
            p_ref[sl][n] = pt
            rl_ref[sl][n] = jnp.broadcast_to(1.0 / l, (8, 2 * R))
            yield

    def gen_pv(sl):
        for p in range(2):
            vp = v_ref[sl][96 * p:96 * p + 96, :]
            res = []
            for (n, v_lo, v_hi) in ((2 * p, vp[0:DH], vp[DH:2 * DH]), (2 * p + 1, vp[DH:2 * DH], vp[0:DH])):
                pt = p_ref[sl][n]
                rhs = jnp.concatenate([jnp.where(l_lt56, pt, 0.0), jnp.where(l_lt56, 0.0, pt)], axis=0)
                lv = jnp.where(l_lt56_d, v_lo, v_hi)
                res.append(_dot(lv, rhs, NN))
                yield
            o0 = res[0] * jnp.concatenate([rl_ref[sl][2 * p]] * (DH // 8), axis=0)
            o1 = res[1] * jnp.concatenate([rl_ref[sl][2 * p + 1]] * (DH // 8), axis=0)
            ot_ref[sl][96 * p:96 * p + DH, 0:2 * R] = jnp.where(l_lt56_d, o0, o1)
            ot_ref[sl][96 * p + DH:96 * p + 2 * DH, 0:2 * R] = jnp.where(l_lt56_d, o1, o0)
            yield

    def gen_d(u, sl, os_ref):
        if not isinstance(u, int):
            u = jnp.where(u >= 0, u, NP)
        ca = u * (2 * WS)
        cb = ca + WS
        for k_, r_lo in ((0, 0), (1, 64)):
            on = ot_ref[sl][r_lo:r_lo + 128, :].T
            yield
            for c_, r0 in ((ca, 0), (cb, R)):
                for i in range(WS):
                    os_ref[i, k_, pl.ds(c_, WS), :] = on[r0 + 8 * i:r0 + 8 * i + WS, :]
            yield

    def gen_half(j, par, hn_ref, kn_ref, os_ref):
        ok = (lambda u: u if 0 <= u < NP else None) if isinstance(j, int) else (lambda u: u)
        for st in HORD:
            if st == 'd' and ok(j - 4) is not None: yield from gen_d(j - 4, par, os_ref)
            if st == 'v' and ok(j - 3) is not None: yield from gen_pv(1 - par)
            if st == 's' and ok(j - 2) is not None: yield from gen_s(j - 2, par, kn_ref)
            if st == 'a': yield from gen_aa(ok(j), par, ok(j - 1), 1 - par, hn_ref)
    N_HALF = 4 + 6 + 8 + 6

    NCONV = C // CG
    assert NP % 2 == 1 and NP // 2 + 1 == NCONV + WS
    x0w = jax.lax.rem(s, 3)
    x0o = jax.lax.rem(s + 1, 3)

    def body(xs_r, xs_w, hn_r, hn_w, kn_r, kn_w, os_w, os_r):
        _interleave((gen_half(0, 0, hn_r, kn_r, os_w), 6))
        nc = NCONV // NB1

        def loop1(it, carry):
            halves = [gen_half(2 * nc * it + 1 + n, (1 + n) % 2, hn_r, kn_r, os_w) for n in range(2 * nc)]
            convs = [conv_gen(nc * it + n, x0w, xs_r) for n in range(nc)]
            _interleave((_chain(*halves), 2 * nc * N_HALF), (_chain(*convs), nc * N_CONV))
            return carry

        jax.lax.fori_loop(0, NB1, loop1, 0)
        j0 = 2 * NCONV + 1
        planes = range(WS)
        rolls = range(C // RG)
        _interleave(
            (_chain(*[gen_half(j, j % 2, hn_r, kn_r, os_w) for j in range(j0, NP + 4)]), (NP + 2 - j0) * N_HALF),
            (_chain(*[_chain(ln_gen(i, x0w, hn_w), kproj_gen(i, hn_w, kn_w)) for i in planes]), WS * (N_LN + N_KP)),
            (_chain(*[out_gen(i, x0o, os_r) for i in planes]), WS * N_OUT),
            (_chain(*[roll_gen(i, xs_w) for i in rolls]), len(rolls) * N_ROLL))

    par = jax.lax.rem(s, 2)

    @pl.when(par == 0)
    def _():
        body(xsa_ref, xsb_ref, hna_ref, hnb_ref, kna_ref, knb_ref, osa_ref, osb_ref)

    @pl.when(par == 1)
    def _():
        body(xsb_ref, xsa_ref, hnb_ref, hna_ref, knb_ref, kna_ref, osb_ref, osa_ref)


@jax.jit
def pallas_standalone__window_attn_davit__vision_kernel(
    x: jax.Array,
    dw_pe: jax.Array,
    w_qkv: jax.Array,
    w_o: jax.Array,
):
    B, H, W, Cc = x.shape
    assert B == 1 and Cc == C and H % WS == 0 and W % WS == 0
    W2 = -(-W // 128) * 128
    nstrip = H // WS
    xt = x.transpose(0, 1, 3, 2)
    dw = dw_pe.reshape(9, C)
    RP = W2 + 32
    out = pl.pallas_call(
        functools.partial(_kernel, W=W, W2=W2, nstrip=nstrip),
        grid=(nstrip + 3,),
        in_specs=[
            pl.BlockSpec((1, WS, C, W2), lambda s: (0, jnp.minimum(s, nstrip - 1), 0, 0)),
            pl.BlockSpec((1, 1, C, W2), lambda s: (0, jnp.clip(s * WS - 1, 0, H - 1), 0, 0)),
            pl.BlockSpec((1, 1, C, W2), lambda s: (0, jnp.minimum(s * WS + WS, H - 1), 0, 0)),
            pl.BlockSpec((9, C), lambda s: (0, 0)),
            pl.BlockSpec((C, 3 * C), lambda s: (0, 0)),
            pl.BlockSpec((C, C), lambda s: (0, 0)),
        ],
        out_specs=pl.BlockSpec((1, WS, C, W2), lambda s: (0, jnp.maximum(s - 3, 0), 0, 0)),
        out_shape=jax.ShapeDtypeStruct((1, H, C, W), x.dtype),
        scratch_shapes=[
            pltpu.VMEM((9, C, 128), F32),
            pltpu.VMEM((2, 2, 64, 128), U32),
            pltpu.VMEM((2, C, 128), U32),
            pltpu.VMEM((2, C // 2, 128), U32),
            pltpu.VMEM((3, WS, C, W2), F32),
            pltpu.VMEM((WS, 2, RP, 128), F32),
            pltpu.VMEM((WS, 2, RP, 128), F32),
            pltpu.VMEM((WS, 2, RP, 128), F32),
            pltpu.VMEM((WS, 2, RP, 128), F32),
            pltpu.VMEM((3, 9, C, W2), BF16),
            pltpu.VMEM((3, 9, C, W2), BF16),
            pltpu.VMEM((WS, 2, RP, 128), F32),
            pltpu.VMEM((WS, 2, RP, 128), F32),
            pltpu.VMEM((C, 112), F32), pltpu.VMEM((C, 112), F32),
            pltpu.VMEM((C, 112), F32), pltpu.VMEM((C, 112), F32),
            pltpu.VMEM((4, 56, 112), F32), pltpu.VMEM((4, 56, 112), F32),
            pltpu.VMEM((4, 8, 112), F32), pltpu.VMEM((4, 8, 112), F32),
            pltpu.VMEM((C, 128), F32), pltpu.VMEM((C, 128), F32),
        ],
        compiler_params=pltpu.CompilerParams(
            dimension_semantics=("arbitrary",), vmem_limit_bytes=100 * 2**20),
        name="davit_window_attn",
    )(xt, xt, xt, dw, w_qkv, w_o)
    return out.transpose(0, 1, 3, 2)
```

```python
import functools
import jax
import jax.numpy as jnp
from jax.experimental import pallas as pl
from jax.experimental.pallas import tpu as pltpu

WS = 7
NH = 4
C = 192
DH = 48
F32 = jnp.float32
BF16 = jnp.bfloat16
NN = (((1,), (0,)), ((), ()))
NT = (((1,), (1,)), ((), ()))
LOG2E = 1.4426950408889634
HORD = 'vsda'
NB1 = 2
CY = 3
U32 = jnp.uint32


def _pk(w):
    return pltpu.bitcast(w.astype(BF16), U32)


def _unpk(w):
    return pltpu.bitcast(w, BF16)


def _dot(a, b, d):
    return jax.lax.dot_general(a, b, d, preferred_element_type=F32)


def _iota(shape, dim):
    return jax.lax.broadcasted_iota(jnp.int32, shape, dim)


def _interleave(*streams):
    items = [[g, n, 0] for g, n in streams]
    while items:
        it = min(items, key=lambda t: (t[2] + 0.5) / t[1])
        try:
            next(it[0])
            it[2] += 1
        except StopIteration:
            items.remove(it)


def _chain(*gens):
    for g in gens:
        yield from g


def _kernel(x_ref, xu_ref, xd_ref, dw_ref, wqkv_ref, wo_ref, o_ref,
            wb_ref, wk_ref, wqv_ref, wot_ref, x0_ref, hna_ref, hnb_ref, osa_ref, osb_ref,
            xsa_ref, xsb_ref, kna_ref, knb_ref, q0, q1, v0, v1, p0, p1, rl0, rl1, ot0, ot1, *, W, W2, nstrip):
    s = pl.program_id(0)
    q_ref, v_ref, p_ref, rl_ref, ot_ref = (q0, q1), (v0, v1), (p0, p1), (rl0, rl1), (ot0, ot1)

    @pl.when(s == 0)
    def _prep():
        dw = dw_ref[...].astype(F32)
        dwp = jnp.concatenate([dw, jnp.zeros((128 - 9, C), F32)], axis=0)
        dwt = dwp.T
        for t in range(9):
            col = dwt[:, t:t + 1]
            if t == 4:
                col = col + 1.0
            wb_ref[t] = jnp.broadcast_to(col, (C, 128))
        w = wqkv_ref[...].astype(F32)
        z = jnp.zeros((C, 32), F32)
        wk = jnp.concatenate([w[:, C:C + 96], z, w[:, C + 96:2 * C], z], axis=1)
        wkp = jnp.concatenate([wk[0:128], jnp.zeros((64, 256), F32), wk[128:C]], axis=0)
        for kt in range(2):
            for nt in range(2):
                wk_ref[kt, nt] = _pk(wkp[128 * kt:128 * kt + 128, 128 * nt:128 * nt + 128])
        wq = w[:, 0:C] * (DH ** -0.5 * LOG2E)
        wqv = jnp.concatenate([wq, w[:, 2 * C:3 * C]], axis=1)
        wqv = jnp.concatenate([wqv[0:128], jnp.zeros((64, 2 * C), F32), wqv[128:C]], axis=0)
        wqv_ref[0] = _pk(wqv[0:128].T)
        wqv_ref[1] = _pk(wqv[128:256].T)
        wo = wo_ref[...].astype(F32)
        wo = jnp.concatenate([wo, jnp.zeros((C, 64), F32)], axis=1)
        wot_ref[0] = _pk(wo[0:128].T[0:C])
        wo1 = jnp.concatenate([jnp.zeros((64, 256), F32), wo[128:C]], axis=0)
        wot_ref[1] = _pk(wo1.T[0:C])
        for r_ in (kna_ref, knb_ref, q0, q1, v0, v1, p0, p1, rl0, rl1, ot0, ot1):
            r_[...] = jnp.zeros(r_.shape, F32)
        for r_ in (hna_ref, hnb_ref, osa_ref, osb_ref, x0_ref):
            r_[...] = jnp.zeros(r_.shape, F32)
        for r_ in (xsa_ref, xsb_ref):
            r_[...] = jnp.zeros(r_.shape, BF16)

    lane = _iota((1, W2), 1)
    cmask = lane < W

    def load_row(r, c0, nc):
        if r == 0:
            v = xu_ref[0, 0, pl.ds(c0, nc), :]
            v = jnp.where(jnp.logical_and(cmask, s > 0), v, jnp.zeros_like(v))
        elif r == 8:
            v = xd_ref[0, 0, pl.ds(c0, nc), :]
            v = jnp.where(jnp.logical_and(cmask, s < nstrip - 1), v, jnp.zeros_like(v))
        else:
            v0 = x_ref[0, r - 1, pl.ds(c0, nc), 0:W2 - 128]
            v1 = x_ref[0, r - 1, pl.ds(c0, nc), W2 - 128:W2]
            v1 = jnp.where(cmask[:, W2 - 128:], v1, jnp.zeros_like(v1))
            v = jnp.concatenate([v0, v1], axis=1)
        return v

    CG = 16

    RG = 32

    def roll_gen(it, xs_ref):
        c0 = it * RG
        if not isinstance(c0, int):
            c0 = pl.multiple_of(c0, RG)
        for r in range(9):
            v = load_row(r, c0, RG)
            xs_ref[1, r, pl.ds(c0, RG), :] = v
            xs_ref[0, r, pl.ds(c0, RG), :] = pltpu.roll(v, 1, 1)
            yield
            xs_ref[2, r, pl.ds(c0, RG), :] = pltpu.roll(v, W2 - 1, 1)
            yield
    N_ROLL = 18

    def conv_gen(g, xs, xs_ref):
        for t in range(W2 // 128):
            ts = slice(t * 128, (t + 1) * 128)
            for hh in range(CG // 8):
                c0 = g * CG + 8 * hh
                if not isinstance(c0, int):
                    c0 = pl.multiple_of(c0, 8)
                wts = [wb_ref[k_, pl.ds(c0, 8), :] for k_ in range(9)]
                acc = [None] * WS
                for r in range(9):
                    sh = [xs_ref[j, r, pl.ds(c0, 8), ts].astype(F32) for j in range(3)]
                    for a in range(3):
                        i = r - a
                        if i < 0 or i >= WS:
                            continue
                        t_ = sh[0] * wts[3 * a] + sh[1] * wts[3 * a + 1] + sh[2] * wts[3 * a + 2]
                        acc[i] = t_ if acc[i] is None else acc[i] + t_
                        if a == 2:
                            x0_ref[xs, i, pl.ds(c0, 8), ts] = acc[i]
                    if r % CY == CY - 1:
                        yield
    N_CONV = 4 * (CG // 8) * (9 // CY)

    def ln_gen(i, xs, hn_ref):
        for t in range(W2 // 128):
            x0 = x0_ref[xs, i, :, t * 128:(t + 1) * 128]
            m = jnp.sum(x0, axis=0, keepdims=True) * (1.0 / C)
            yield
            xc = x0 - m
            var = jnp.sum(xc * xc, axis=0, keepdims=True) * (1.0 / C)
            yield
            h = xc * jax.lax.rsqrt(var + 1e-5)
            ht0 = h[0:128].T
            yield
            hn_ref[i, 0, t * 128:(t + 1) * 128, :] = ht0
            ht1 = h[64:C].T
            yield
            hn_ref[i, 1, t * 128:(t + 1) * 128, :] = ht1
            yield
    N_LN = 5 * 4

    def kproj_gen(i, hn_ref, kn_ref):
        for t in range(W2 // 128):
            ht0 = hn_ref[i, 0, t * 128:(t + 1) * 128, :]
            ht1 = hn_ref[i, 1, t * 128:(t + 1) * 128, :]
            d = []
            for nt in range(2):
                d.append(_dot(ht0, _unpk(wk_ref[0, nt]), NN))
                yield
                d.append(_dot(ht1, _unpk(wk_ref[1, nt]), NN))
                yield
            for nt in range(2):
                kn_ref[i, nt, t * 128:(t + 1) * 128, :] = d[2 * nt] + d[2 * nt + 1]
                yield
    N_KP = 6 * 4

    def out_gen(i, xs, os_ref):
        for t in range(W2 // 128):
            y0 = _dot(_unpk(wot_ref[0]), os_ref[i, 0, t * 128:(t + 1) * 128, :], NT)
            yield
            y1 = _dot(_unpk(wot_ref[1]), os_ref[i, 1, t * 128:(t + 1) * 128, :], NT)
            yield
            y = (y0 + y1) + x0_ref[xs, i, :, t * 128:(t + 1) * 128]
            o_ref[0, i, :, t * 128:(t + 1) * 128] = y.astype(o_ref.dtype)
            yield
    N_OUT = 3 * 4

    R = 8 * WS
    lane128 = _iota((R, 128), 1)
    l_lt48 = lane128 < DH
    lane112 = _iota((R, 2 * R), 1)
    l_lt56 = lane112 < R
    rowvalid = (_iota((R, 2 * R), 0) & 7) != 7
    mq = (_iota((2 * DH, 2 * R), 0) < DH) == (_iota((2 * DH, 2 * R), 1) < R)
    l_lt56_d = _iota((DH, 2 * R), 1) < R
    NP = (W // WS + 1) // 2

    def gen_a(u, part, dst_ref, hn_ref):
        ca = u * (2 * WS)
        cb = ca + WS
        hw0 = jnp.concatenate([hn_ref[i, 0, pl.ds(c_, 8), :] for c_ in (ca, cb) for i in range(WS)], axis=0)
        hw1 = jnp.concatenate([hn_ref[i, 1, pl.ds(c_, 8), :] for c_ in (ca, cb) for i in range(WS)], axis=0)
        hf = C // 2
        d0 = _dot(_unpk(wqv_ref[0, part * hf:(part + 1) * hf]), hw0, NT)
        yield
        d1 = _dot(_unpk(wqv_ref[1, part * hf:(part + 1) * hf]), hw1, NT)
        yield
        return d0, d1, dst_ref

    def gen_aa(uq, slq, uv, slv, hn_ref):
        rq = rv = None
        if uq is not None:
            rq = yield from gen_a(uq, 0, q_ref[slq], hn_ref)
        if uv is not None:
            rv = yield from gen_a(uv, 1, v_ref[slv], hn_ref)
        if rq is not None:
            rq[2][...] = rq[0] + rq[1]
        yield
        if rv is not None:
            rv[2][...] = rv[0] + rv[1]
        yield

    def gen_s(u, sl, kn_ref):
        if not isinstance(u, int):
            u = jnp.maximum(u, 0)
        ca = u * (2 * WS)
        cb = ca + WS
        sts = []
        for p in range(2):
            qp = q_ref[sl][96 * p:96 * p + 96, :]
            ka = jnp.concatenate([kn_ref[i, p, pl.ds(ca, 8), :] for i in range(WS)], axis=0)
            kb = jnp.concatenate([kn_ref[i, p, pl.ds(cb, 8), :] for i in range(WS)], axis=0)
            lx = jnp.where(l_lt48, ka, kb)[:, 0:96]
            rx = jnp.where(mq, qp, 0.0)
            sts.append(_dot(lx, rx, NN))
            yield
            ly = jnp.where(l_lt48, kb, ka)[:, 0:96]
            ry = jnp.where(mq, 0.0, qp)
            sts.append(_dot(ly, ry, NN))
            yield
        for n, st in enumerate(sts):
            st = jnp.where(rowvalid, st, -jnp.inf)
            mx = jnp.max(st, axis=0, keepdims=True)
            pt = jnp.exp2(st - mx)
            l = jnp.sum(pt, axis=0, keepdims=True)
            p_ref[sl][n] = pt
            rl_ref[sl][n] = jnp.broadcast_to(1.0 / l, (8, 2 * R))
            yield

    def gen_pv(sl):
        for p in range(2):
            vp = v_ref[sl][96 * p:96 * p + 96, :]
            res = []
            for (n, v_lo, v_hi) in ((2 * p, vp[0:DH], vp[DH:2 * DH]), (2 * p + 1, vp[DH:2 * DH], vp[0:DH])):
                pt = p_ref[sl][n]
                rhs = jnp.concatenate([jnp.where(l_lt56, pt, 0.0), jnp.where(l_lt56, 0.0, pt)], axis=0)
                lv = jnp.where(l_lt56_d, v_lo, v_hi)
                res.append(_dot(lv, rhs, NN))
                yield
            o0 = res[0] * jnp.concatenate([rl_ref[sl][2 * p]] * (DH // 8), axis=0)
            o1 = res[1] * jnp.concatenate([rl_ref[sl][2 * p + 1]] * (DH // 8), axis=0)
            ot_ref[sl][96 * p:96 * p + DH, 0:2 * R] = jnp.where(l_lt56_d, o0, o1)
            ot_ref[sl][96 * p + DH:96 * p + 2 * DH, 0:2 * R] = jnp.where(l_lt56_d, o1, o0)
            yield

    def gen_d(u, sl, os_ref):
        if not isinstance(u, int):
            u = jnp.where(u >= 0, u, NP)
        ca = u * (2 * WS)
        cb = ca + WS
        for k_, r_lo in ((0, 0), (1, 64)):
            on = ot_ref[sl][r_lo:r_lo + 128, :].T
            yield
            for c_, r0 in ((ca, 0), (cb, R)):
                for i in range(WS):
                    os_ref[i, k_, pl.ds(c_, WS), :] = on[r0 + 8 * i:r0 + 8 * i + WS, :]
            yield

    def gen_half(j, par, hn_ref, kn_ref, os_ref):
        ok = (lambda u: u if 0 <= u < NP else None) if isinstance(j, int) else (lambda u: u)
        for st in HORD:
            if st == 'd' and ok(j - 4) is not None: yield from gen_d(j - 4, par, os_ref)
            if st == 'v' and ok(j - 3) is not None: yield from gen_pv(1 - par)
            if st == 's' and ok(j - 2) is not None: yield from gen_s(j - 2, par, kn_ref)
            if st == 'a': yield from gen_aa(ok(j), par, ok(j - 1), 1 - par, hn_ref)
    N_HALF = 4 + 6 + 8 + 6

    NCONV = C // CG
    assert NP % 2 == 1 and NP // 2 + 1 == NCONV + WS
    x0w = jax.lax.rem(s, 3)
    x0o = jax.lax.rem(s + 1, 3)

    def body(xs_r, xs_w, hn_r, hn_w, kn_r, kn_w, os_w, os_r):
        nc = NCONV // NB1

        def loop1(it, carry):
            halves = [gen_half(2 * nc * it + 1 + n, (1 + n) % 2, hn_r, kn_r, os_w) for n in range(2 * nc)]
            convs = [conv_gen(nc * it + n, x0w, xs_r) for n in range(nc)]
            _interleave((_chain(*halves), 2 * nc * N_HALF), (_chain(*convs), nc * N_CONV))
            return carry

        j0 = 2 * NCONV + 1
        planes = range(WS)
        rolls = range(C // RG)

        @pl.when(s <= 1)
        def _():
            def item(it, carry):
                _interleave((roll_gen(it, xs_w), N_ROLL))
                return carry
            jax.lax.fori_loop(0, C // RG, item, 0)

        @pl.when(s == 1)
        def _():
            def conv_item(g, carry):
                _interleave((conv_gen(g, x0w, xs_r), N_CONV))
                return carry
            jax.lax.fori_loop(0, NCONV, conv_item, 0)

            def ln_item(i, carry):
                _interleave((ln_gen(i, x0w, hn_w), N_LN))
                return carry
            jax.lax.fori_loop(0, WS, ln_item, 0)

            def k_item(i, carry):
                _interleave((kproj_gen(i, hn_w, kn_w), N_KP))
                return carry
            jax.lax.fori_loop(0, WS, k_item, 0)

        @pl.when(s == nstrip + 2)
        def _():
            def item(i, carry):
                _interleave((out_gen(i, x0o, os_r), N_OUT))
                return carry
            jax.lax.fori_loop(0, WS, item, 0)

        @pl.when(jnp.logical_and(s > 1, s < nstrip + 2))
        def _():
            _interleave((gen_half(0, 0, hn_r, kn_r, os_w), 6))
            jax.lax.fori_loop(0, NB1, loop1, 0)
            _interleave(
                (_chain(*[gen_half(j, j % 2, hn_r, kn_r, os_w) for j in range(j0, NP + 4)]), (NP + 2 - j0) * N_HALF),
                (_chain(*[_chain(ln_gen(i, x0w, hn_w), kproj_gen(i, hn_w, kn_w)) for i in planes]),
                 WS * (N_LN + N_KP)),
                (_chain(*[out_gen(i, x0o, os_r) for i in planes]), WS * N_OUT),
                (_chain(*[roll_gen(i, xs_w) for i in rolls]), len(rolls) * N_ROLL))

    par = jax.lax.rem(s, 2)

    @pl.when(par == 0)
    def _():
        body(xsa_ref, xsb_ref, hna_ref, hnb_ref, kna_ref, knb_ref, osa_ref, osb_ref)

    @pl.when(par == 1)
    def _():
        body(xsb_ref, xsa_ref, hnb_ref, hna_ref, knb_ref, kna_ref, osb_ref, osa_ref)


@jax.jit
def pallas_standalone__window_attn_davit__vision_kernel(
    x: jax.Array,
    dw_pe: jax.Array,
    w_qkv: jax.Array,
    w_o: jax.Array,
):
    B, H, W, Cc = x.shape
    assert B == 1 and Cc == C and H % WS == 0 and W % WS == 0
    W2 = -(-W // 128) * 128
    nstrip = H // WS
    xt = x.transpose(0, 1, 3, 2)
    dw = dw_pe.reshape(9, C)
    RP = W2 + 32
    out = pl.pallas_call(
        functools.partial(_kernel, W=W, W2=W2, nstrip=nstrip),
        grid=(nstrip + 3,),
        in_specs=[
            pl.BlockSpec((1, WS, C, W2), lambda s: (0, jnp.minimum(s, nstrip - 1), 0, 0)),
            pl.BlockSpec((1, 1, C, W2), lambda s: (0, jnp.clip(s * WS - 1, 0, H - 1), 0, 0)),
            pl.BlockSpec((1, 1, C, W2), lambda s: (0, jnp.minimum(s * WS + WS, H - 1), 0, 0)),
            pl.BlockSpec((9, C), lambda s: (0, 0)),
            pl.BlockSpec((C, 3 * C), lambda s: (0, 0)),
            pl.BlockSpec((C, C), lambda s: (0, 0)),
        ],
        out_specs=pl.BlockSpec((1, WS, C, W2), lambda s: (0, jnp.maximum(s - 3, 0), 0, 0)),
        out_shape=jax.ShapeDtypeStruct((1, H, C, W), x.dtype),
        scratch_shapes=[
            pltpu.VMEM((9, C, 128), F32),
            pltpu.VMEM((2, 2, 64, 128), U32),
            pltpu.VMEM((2, C, 128), U32),
            pltpu.VMEM((2, C // 2, 128), U32),
            pltpu.VMEM((3, WS, C, W2), F32),
            pltpu.VMEM((WS, 2, RP, 128), F32),
            pltpu.VMEM((WS, 2, RP, 128), F32),
            pltpu.VMEM((WS, 2, RP, 128), F32),
            pltpu.VMEM((WS, 2, RP, 128), F32),
            pltpu.VMEM((3, 9, C, W2), BF16),
            pltpu.VMEM((3, 9, C, W2), BF16),
            pltpu.VMEM((WS, 2, RP, 128), F32),
            pltpu.VMEM((WS, 2, RP, 128), F32),
            pltpu.VMEM((C, 112), F32), pltpu.VMEM((C, 112), F32),
            pltpu.VMEM((C, 112), F32), pltpu.VMEM((C, 112), F32),
            pltpu.VMEM((4, 56, 112), F32), pltpu.VMEM((4, 56, 112), F32),
            pltpu.VMEM((4, 8, 112), F32), pltpu.VMEM((4, 8, 112), F32),
            pltpu.VMEM((C, 128), F32), pltpu.VMEM((C, 128), F32),
        ],
        compiler_params=pltpu.CompilerParams(
            dimension_semantics=("arbitrary",), vmem_limit_bytes=100 * 2**20),
        name="davit_window_attn",
    )(xt, xt, xt, dw, w_qkv, w_o)
    return out.transpose(0, 1, 3, 2)
```

```python
import functools
import jax
import jax.numpy as jnp
from jax.experimental import pallas as pl
from jax.experimental.pallas import tpu as pltpu

WS = 7
NH = 4
C = 192
DH = 48
F32 = jnp.float32
BF16 = jnp.bfloat16
NN = (((1,), (0,)), ((), ()))
NT = (((1,), (1,)), ((), ()))
LOG2E = 1.4426950408889634
HORD = 'vsda'
NH1 = 20
NB1 = 2
CY = 3
U32 = jnp.uint32


def _pk(w):
    return pltpu.bitcast(w.astype(BF16), U32)


def _unpk(w):
    return pltpu.bitcast(w, BF16)


def _dot(a, b, d):
    return jax.lax.dot_general(a, b, d, preferred_element_type=F32)


def _iota(shape, dim):
    return jax.lax.broadcasted_iota(jnp.int32, shape, dim)


def _interleave(*streams):
    items = [[g, n, 0] for g, n in streams]
    while items:
        it = min(items, key=lambda t: (t[2] + 0.5) / t[1])
        try:
            next(it[0])
            it[2] += 1
        except StopIteration:
            items.remove(it)


def _chain(*gens):
    for g in gens:
        yield from g


def _kernel(x_ref, xu_ref, xd_ref, dw_ref, wqkv_ref, wo_ref, o_ref,
            wb_ref, wk_ref, wqv_ref, wot_ref, x0_ref, hna_ref, hnb_ref, osa_ref, osb_ref,
            xsa_ref, xsb_ref, kna_ref, knb_ref, q0, q1, v0, v1, p0, p1, rl0, rl1, ot0, ot1, *, W, W2, nstrip):
    s = pl.program_id(0)
    q_ref, v_ref, p_ref, rl_ref, ot_ref = (q0, q1), (v0, v1), (p0, p1), (rl0, rl1), (ot0, ot1)

    @pl.when(s == 0)
    def _prep():
        dw = dw_ref[...].astype(F32)
        dwp = jnp.concatenate([dw, jnp.zeros((128 - 9, C), F32)], axis=0)
        dwt = dwp.T
        for t in range(9):
            col = dwt[:, t:t + 1]
            if t == 4:
                col = col + 1.0
            wb_ref[t] = jnp.broadcast_to(col, (C, 128))
        w = wqkv_ref[...].astype(F32)
        z = jnp.zeros((C, 32), F32)
        wk = jnp.concatenate([w[:, C:C + 96], z, w[:, C + 96:2 * C], z], axis=1)
        wkp = jnp.concatenate([wk[0:128], jnp.zeros((64, 256), F32), wk[128:C]], axis=0)
        for kt in range(2):
            for nt in range(2):
                wk_ref[kt, nt] = _pk(wkp[128 * kt:128 * kt + 128, 128 * nt:128 * nt + 128])
        wq = w[:, 0:C] * (DH ** -0.5 * LOG2E)
        wqv = jnp.concatenate([wq, w[:, 2 * C:3 * C]], axis=1)
        wqv = jnp.concatenate([wqv[0:128], jnp.zeros((64, 2 * C), F32), wqv[128:C]], axis=0)
        wqv_ref[0] = _pk(wqv[0:128].T)
        wqv_ref[1] = _pk(wqv[128:256].T)
        wo = wo_ref[...].astype(F32)
        wo = jnp.concatenate([wo, jnp.zeros((C, 64), F32)], axis=1)
        wot_ref[0] = _pk(wo[0:128].T[0:C])
        wo1 = jnp.concatenate([jnp.zeros((64, 256), F32), wo[128:C]], axis=0)
        wot_ref[1] = _pk(wo1.T[0:C])
        for r_ in (kna_ref, knb_ref, q0, q1, v0, v1, p0, p1, rl0, rl1, ot0, ot1):
            r_[...] = jnp.zeros(r_.shape, F32)
        for r_ in (hna_ref, hnb_ref, osa_ref, osb_ref, x0_ref):
            r_[...] = jnp.zeros(r_.shape, F32)
        for r_ in (xsa_ref, xsb_ref):
            r_[...] = jnp.zeros(r_.shape, BF16)

    lane = _iota((1, W2), 1)
    cmask = lane < W

    def load_row(r, c0, nc):
        if r == 0:
            v = xu_ref[0, 0, pl.ds(c0, nc), :]
            v = jnp.where(jnp.logical_and(cmask, s > 0), v, jnp.zeros_like(v))
        elif r == 8:
            v = xd_ref[0, 0, pl.ds(c0, nc), :]
            v = jnp.where(jnp.logical_and(cmask, s < nstrip - 1), v, jnp.zeros_like(v))
        else:
            v0 = x_ref[0, r - 1, pl.ds(c0, nc), 0:W2 - 128]
            v1 = x_ref[0, r - 1, pl.ds(c0, nc), W2 - 128:W2]
            v1 = jnp.where(cmask[:, W2 - 128:], v1, jnp.zeros_like(v1))
            v = jnp.concatenate([v0, v1], axis=1)
        return v

    CG = 16

    RG = 32

    def roll_gen(it, xs_ref):
        c0 = it * RG
        if not isinstance(c0, int):
            c0 = pl.multiple_of(c0, RG)
        for r in range(9):
            v = load_row(r, c0, RG)
            xs_ref[1, r, pl.ds(c0, RG), :] = v
            xs_ref[0, r, pl.ds(c0, RG), :] = pltpu.roll(v, 1, 1)
            yield
            xs_ref[2, r, pl.ds(c0, RG), :] = pltpu.roll(v, W2 - 1, 1)
            yield
    N_ROLL = 18

    def conv_gen(g, xs, xs_ref):
        for t in range(W2 // 128):
            ts = slice(t * 128, (t + 1) * 128)
            for hh in range(CG // 8):
                c0 = g * CG + 8 * hh
                if not isinstance(c0, int):
                    c0 = pl.multiple_of(c0, 8)
                wts = [wb_ref[k_, pl.ds(c0, 8), :] for k_ in range(9)]
                acc = [None] * WS
                for r in range(9):
                    sh = [xs_ref[j, r, pl.ds(c0, 8), ts].astype(F32) for j in range(3)]
                    for a in range(3):
                        i = r - a
                        if i < 0 or i >= WS:
                            continue
                        t_ = sh[0] * wts[3 * a] + sh[1] * wts[3 * a + 1] + sh[2] * wts[3 * a + 2]
                        acc[i] = t_ if acc[i] is None else acc[i] + t_
                        if a == 2:
                            x0_ref[xs, i, pl.ds(c0, 8), ts] = acc[i]
                    if r % CY == CY - 1:
                        yield
    N_CONV = 4 * (CG // 8) * (9 // CY)

    def ln_gen(i, xs, hn_ref):
        for t in range(W2 // 128):
            x0 = x0_ref[xs, i, :, t * 128:(t + 1) * 128]
            m = jnp.sum(x0, axis=0, keepdims=True) * (1.0 / C)
            yield
            xc = x0 - m
            var = jnp.sum(xc * xc, axis=0, keepdims=True) * (1.0 / C)
            yield
            h = xc * jax.lax.rsqrt(var + 1e-5)
            ht0 = h[0:128].T
            yield
            hn_ref[i, 0, t * 128:(t + 1) * 128, :] = ht0
            ht1 = h[64:C].T
            yield
            hn_ref[i, 1, t * 128:(t + 1) * 128, :] = ht1
            yield
    N_LN = 5 * 4

    def kproj_gen(i, hn_ref, kn_ref):
        for t in range(W2 // 128):
            ht0 = hn_ref[i, 0, t * 128:(t + 1) * 128, :]
            ht1 = hn_ref[i, 1, t * 128:(t + 1) * 128, :]
            d = []
            for nt in range(2):
                d.append(_dot(ht0, _unpk(wk_ref[0, nt]), NN))
                yield
                d.append(_dot(ht1, _unpk(wk_ref[1, nt]), NN))
                yield
            for nt in range(2):
                kn_ref[i, nt, t * 128:(t + 1) * 128, :] = d[2 * nt] + d[2 * nt + 1]
                yield
    N_KP = 6 * 4

    def out_gen(i, xs, os_ref):
        for t in range(W2 // 128):
            y0 = _dot(_unpk(wot_ref[0]), os_ref[i, 0, t * 128:(t + 1) * 128, :], NT)
            yield
            y1 = _dot(_unpk(wot_ref[1]), os_ref[i, 1, t * 128:(t + 1) * 128, :], NT)
            yield
            y = (y0 + y1) + x0_ref[xs, i, :, t * 128:(t + 1) * 128]
            o_ref[0, i, :, t * 128:(t + 1) * 128] = y.astype(o_ref.dtype)
            yield
    N_OUT = 3 * 4

    R = 8 * WS
    lane128 = _iota((R, 128), 1)
    l_lt48 = lane128 < DH
    lane112 = _iota((R, 2 * R), 1)
    l_lt56 = lane112 < R
    rowvalid = (_iota((R, 2 * R), 0) & 7) != 7
    mq = (_iota((2 * DH, 2 * R), 0) < DH) == (_iota((2 * DH, 2 * R), 1) < R)
    l_lt56_d = _iota((DH, 2 * R), 1) < R
    NP = (W // WS + 1) // 2

    def gen_a(u, part, dst_ref, hn_ref):
        ca = u * (2 * WS)
        cb = ca + WS
        hw0 = jnp.concatenate([hn_ref[i, 0, pl.ds(c_, 8), :] for c_ in (ca, cb) for i in range(WS)], axis=0)
        hw1 = jnp.concatenate([hn_ref[i, 1, pl.ds(c_, 8), :] for c_ in (ca, cb) for i in range(WS)], axis=0)
        hf = C // 2
        d0 = _dot(_unpk(wqv_ref[0, part * hf:(part + 1) * hf]), hw0, NT)
        yield
        d1 = _dot(_unpk(wqv_ref[1, part * hf:(part + 1) * hf]), hw1, NT)
        yield
        return d0, d1, dst_ref

    def gen_aa(uq, slq, uv, slv, hn_ref):
        rq = rv = None
        if uq is not None:
            rq = yield from gen_a(uq, 0, q_ref[slq], hn_ref)
        if uv is not None:
            rv = yield from gen_a(uv, 1, v_ref[slv], hn_ref)
        if rq is not None:
            rq[2][...] = rq[0] + rq[1]
        yield
        if rv is not None:
            rv[2][...] = rv[0] + rv[1]
        yield

    def gen_s(u, sl, kn_ref):
        if not isinstance(u, int):
            u = jnp.maximum(u, 0)
        ca = u * (2 * WS)
        cb = ca + WS
        sts = []
        for p in range(2):
            qp = q_ref[sl][96 * p:96 * p + 96, :]
            ka = jnp.concatenate([kn_ref[i, p, pl.ds(ca, 8), :] for i in range(WS)], axis=0)
            kb = jnp.concatenate([kn_ref[i, p, pl.ds(cb, 8), :] for i in range(WS)], axis=0)
            lx = jnp.where(l_lt48, ka, kb)[:, 0:96]
            rx = jnp.where(mq, qp, 0.0)
            sts.append(_dot(lx, rx, NN))
            yield
            ly = jnp.where(l_lt48, kb, ka)[:, 0:96]
            ry = jnp.where(mq, 0.0, qp)
            sts.append(_dot(ly, ry, NN))
            yield
        for n, st in enumerate(sts):
            st = jnp.where(rowvalid, st, -jnp.inf)
            mx = jnp.max(st, axis=0, keepdims=True)
            pt = jnp.exp2(st - mx)
            l = jnp.sum(pt, axis=0, keepdims=True)
            p_ref[sl][n] = pt
            rl_ref[sl][n] = jnp.broadcast_to(1.0 / l, (8, 2 * R))
            yield

    def gen_pv(sl):
        for p in range(2):
            vp = v_ref[sl][96 * p:96 * p + 96, :]
            res = []
            for (n, v_lo, v_hi) in ((2 * p, vp[0:DH], vp[DH:2 * DH]), (2 * p + 1, vp[DH:2 * DH], vp[0:DH])):
                pt = p_ref[sl][n]
                rhs = jnp.concatenate([jnp.where(l_lt56, pt, 0.0), jnp.where(l_lt56, 0.0, pt)], axis=0)
                lv = jnp.where(l_lt56_d, v_lo, v_hi)
                res.append(_dot(lv, rhs, NN))
                yield
            o0 = res[0] * jnp.concatenate([rl_ref[sl][2 * p]] * (DH // 8), axis=0)
            o1 = res[1] * jnp.concatenate([rl_ref[sl][2 * p + 1]] * (DH // 8), axis=0)
            ot_ref[sl][96 * p:96 * p + DH, 0:2 * R] = jnp.where(l_lt56_d, o0, o1)
            ot_ref[sl][96 * p + DH:96 * p + 2 * DH, 0:2 * R] = jnp.where(l_lt56_d, o1, o0)
            yield

    def gen_d(u, sl, os_ref):
        if not isinstance(u, int):
            u = jnp.where(u >= 0, u, NP)
        ca = u * (2 * WS)
        cb = ca + WS
        for k_, r_lo in ((0, 0), (1, 64)):
            on = ot_ref[sl][r_lo:r_lo + 128, :].T
            yield
            for c_, r0 in ((ca, 0), (cb, R)):
                for i in range(WS):
                    os_ref[i, k_, pl.ds(c_, WS), :] = on[r0 + 8 * i:r0 + 8 * i + WS, :]
            yield

    def gen_half(j, par, hn_ref, kn_ref, os_ref):
        ok = (lambda u: u if 0 <= u < NP else None) if isinstance(j, int) else (lambda u: u)
        for st in HORD:
            if st == 'd' and ok(j - 4) is not None: yield from gen_d(j - 4, par, os_ref)
            if st == 'v' and ok(j - 3) is not None: yield from gen_pv(1 - par)
            if st == 's' and ok(j - 2) is not None: yield from gen_s(j - 2, par, kn_ref)
            if st == 'a': yield from gen_aa(ok(j), par, ok(j - 1), 1 - par, hn_ref)
    N_HALF = 4 + 6 + 8 + 6

    NCONV = C // CG
    assert NP % 2 == 1 and NP // 2 + 1 == NCONV + WS
    assert NH1 % (2 * NB1) == 0 and NCONV % NB1 == 0 and NH1 < NP
    x0w = jax.lax.rem(s, 3)
    x0o = jax.lax.rem(s + 1, 3)

    def body(xs_r, xs_w, hn_r, hn_w, kn_r, kn_w, os_w, os_r):
        nc = NCONV // NB1

        def loop1(it, carry):
            nh = NH1 // NB1
            halves = [gen_half(nh * it + 1 + n, (1 + n) % 2, hn_r, kn_r, os_w) for n in range(nh)]
            convs = [conv_gen(nc * it + n, x0w, xs_r) for n in range(nc)]
            _interleave((_chain(*halves), nh * N_HALF), (_chain(*convs), nc * N_CONV))
            return carry

        j0 = NH1 + 1
        planes = range(WS)
        rolls = range(C // RG)

        @pl.when(s <= 1)
        def _():
            def item(it, carry):
                _interleave((roll_gen(it, xs_w), N_ROLL))
                return carry
            jax.lax.fori_loop(0, C // RG, item, 0)

        @pl.when(s == 1)
        def _():
            def conv_item(g, carry):
                _interleave((conv_gen(g, x0w, xs_r), N_CONV))
                return carry
            jax.lax.fori_loop(0, NCONV, conv_item, 0)

            def ln_item(i, carry):
                _interleave((ln_gen(i, x0w, hn_w), N_LN))
                return carry
            jax.lax.fori_loop(0, WS, ln_item, 0)

            def k_item(i, carry):
                _interleave((kproj_gen(i, hn_w, kn_w), N_KP))
                return carry
            jax.lax.fori_loop(0, WS, k_item, 0)

        @pl.when(s == nstrip + 2)
        def _():
            def item(i, carry):
                _interleave((out_gen(i, x0o, os_r), N_OUT))
                return carry
            jax.lax.fori_loop(0, WS, item, 0)

        @pl.when(jnp.logical_and(s > 1, s < nstrip + 2))
        def _():
            _interleave((gen_half(0, 0, hn_r, kn_r, os_w), 6))
            jax.lax.fori_loop(0, NB1, loop1, 0)
            _interleave(
                (_chain(*[gen_half(j, j % 2, hn_r, kn_r, os_w) for j in range(j0, NP + 4)]), (NP + 2 - j0) * N_HALF),
                (_chain(*[_chain(ln_gen(i, x0w, hn_w), kproj_gen(i, hn_w, kn_w)) for i in planes]),
                 WS * (N_LN + N_KP)),
                (_chain(*[out_gen(i, x0o, os_r) for i in planes]), WS * N_OUT),
                (_chain(*[roll_gen(i, xs_w) for i in rolls]), len(rolls) * N_ROLL))

    par = jax.lax.rem(s, 2)

    @pl.when(par == 0)
    def _():
        body(xsa_ref, xsb_ref, hna_ref, hnb_ref, kna_ref, knb_ref, osa_ref, osb_ref)

    @pl.when(par == 1)
    def _():
        body(xsb_ref, xsa_ref, hnb_ref, hna_ref, knb_ref, kna_ref, osb_ref, osa_ref)


@jax.jit
def pallas_standalone__window_attn_davit__vision_kernel(
    x: jax.Array,
    dw_pe: jax.Array,
    w_qkv: jax.Array,
    w_o: jax.Array,
):
    B, H, W, Cc = x.shape
    assert B == 1 and Cc == C and H % WS == 0 and W % WS == 0
    W2 = -(-W // 128) * 128
    nstrip = H // WS
    xt = x.transpose(0, 1, 3, 2)
    dw = dw_pe.reshape(9, C)
    RP = W2 + 32
    out = pl.pallas_call(
        functools.partial(_kernel, W=W, W2=W2, nstrip=nstrip),
        grid=(nstrip + 3,),
        in_specs=[
            pl.BlockSpec((1, WS, C, W2), lambda s: (0, jnp.minimum(s, nstrip - 1), 0, 0)),
            pl.BlockSpec((1, 1, C, W2), lambda s: (0, jnp.clip(s * WS - 1, 0, H - 1), 0, 0)),
            pl.BlockSpec((1, 1, C, W2), lambda s: (0, jnp.minimum(s * WS + WS, H - 1), 0, 0)),
            pl.BlockSpec((9, C), lambda s: (0, 0)),
            pl.BlockSpec((C, 3 * C), lambda s: (0, 0)),
            pl.BlockSpec((C, C), lambda s: (0, 0)),
        ],
        out_specs=pl.BlockSpec((1, WS, C, W2), lambda s: (0, jnp.maximum(s - 3, 0), 0, 0)),
        out_shape=jax.ShapeDtypeStruct((1, H, C, W), x.dtype),
        scratch_shapes=[
            pltpu.VMEM((9, C, 128), F32),
            pltpu.VMEM((2, 2, 64, 128), U32),
            pltpu.VMEM((2, C, 128), U32),
            pltpu.VMEM((2, C // 2, 128), U32),
            pltpu.VMEM((3, WS, C, W2), F32),
            pltpu.VMEM((WS, 2, RP, 128), F32),
            pltpu.VMEM((WS, 2, RP, 128), F32),
            pltpu.VMEM((WS, 2, RP, 128), F32),
            pltpu.VMEM((WS, 2, RP, 128), F32),
            pltpu.VMEM((3, 9, C, W2), BF16),
            pltpu.VMEM((3, 9, C, W2), BF16),
            pltpu.VMEM((WS, 2, RP, 128), F32),
            pltpu.VMEM((WS, 2, RP, 128), F32),
            pltpu.VMEM((C, 112), F32), pltpu.VMEM((C, 112), F32),
            pltpu.VMEM((C, 112), F32), pltpu.VMEM((C, 112), F32),
            pltpu.VMEM((4, 56, 112), F32), pltpu.VMEM((4, 56, 112), F32),
            pltpu.VMEM((4, 8, 112), F32), pltpu.VMEM((4, 8, 112), F32),
            pltpu.VMEM((C, 128), F32), pltpu.VMEM((C, 128), F32),
        ],
        compiler_params=pltpu.CompilerParams(
            dimension_semantics=("arbitrary",), vmem_limit_bytes=100 * 2**20),
        name="davit_window_attn",
    )(xt, xt, xt, dw, w_qkv, w_o)
    return out.transpose(0, 1, 3, 2)
```
